```python
import jax
import jax.numpy as jnp

def _softmax(x, axis=-1):
    return jax.nn.softmax(x, axis=axis)
def _gelu(x):
    return jax.nn.gelu(x, approximate=True)
def _silu(x):
    return jax.nn.silu(x)
def _sigmoid(x):
    return jax.nn.sigmoid(x)
def _layernorm(x, axis=-1, eps=1e-5):
    m = jnp.mean(x, axis=axis, keepdims=True)
    v = jnp.var(x, axis=axis, keepdims=True)
    return (x - m) / jnp.sqrt(v + eps)
def _scatter_add(tgt, idx, src, axis=0):
    return tgt.at[idx].add(src)
def _segment_sum(src, seg, n):
    return jax.ops.segment_sum(src, seg, n)
class _Rng:
    def __init__(self, key):
        self._k = key
    def _next(self):
        self._k, sub = jax.random.split(self._k)
        return sub
    def normal(self, shape):
        return jax.random.normal(self._next(), shape, dtype=jnp.bfloat16)
    def randint(self, lo, hi, shape):
        return jax.random.randint(self._next(), shape, lo, hi, dtype=jnp.int32)
    def uniform(self, shape, lo=0.0, hi=1.0):
        return jax.random.uniform(self._next(), shape, jnp.bfloat16, lo, hi)
    def permutation(self, n):
        return jax.random.permutation(self._next(), n)


kernel_name = 'sequential_preLN__mha_block_cached__moe_arch_mod__decode'

def setup_inputs():
    _rng = _Rng(jax.random.key(int.from_bytes(__import__("os").urandom(4), "little")))
    _w = (lambda a: (lambda t: t.astype(jnp.bfloat16) if jnp.issubdtype(t.dtype, jnp.floating) else t)(jnp.asarray(a)))
    def _A_setup():
        B, Sq, D = 4, 1, 640
        H, Sk, Dh = 32, 8192, 192
        return {
            "x": _w((lambda *s: _rng.normal(s) * 0.05)(B, Sq, D)),
            "k_cache": _w((lambda *s: _rng.normal(s) * 0.05)(B, H, Sk, Dh)),
            "v_cache": _w((lambda *s: _rng.normal(s) * 0.05)(B, H, Sk, Dh)),
            "wq": _w((lambda *s: _rng.normal(s) * 0.05)(D, H * Dh) * (D ** -0.5)),
            "wo": _w((lambda *s: _rng.normal(s) * 0.05)(H * Dh, D) * ((H * Dh) ** -0.5)),
        }
    _A_in = _A_setup()

    def _B_setup():
        B, S, D, F, C = 4, 1, 640, 1536, 1
        return {
            "x": _w((lambda *s: _rng.normal(s) * 0.05)(B, S, D)),
            "w_r": _w((lambda *s: _rng.normal(s) * 0.05)(D)),
            "w_gate": _w((lambda *s: _rng.normal(s) * 0.05)(D, F)),
            "w_up": _w((lambda *s: _rng.normal(s) * 0.05)(D, F)),
            "w_down": _w((lambda *s: _rng.normal(s) * 0.05)(F, D)),
        }
    _B_in = _B_setup()

    return {
        "A_x": _A_in["x"],
        "A_k_cache": _A_in["k_cache"],
        "A_v_cache": _A_in["v_cache"],
        "A_wq": _A_in["wq"],
        "A_wo": _A_in["wo"],
        "B_x": _B_in["x"],
        "B_w_r": _B_in["w_r"],
        "B_w_gate": _B_in["w_gate"],
        "B_w_up": _B_in["w_up"],
        "B_w_down": _B_in["w_down"],
    }

def reference(A_x, A_k_cache, A_v_cache, A_wq, A_wo, B_x, B_w_r, B_w_gate, B_w_up, B_w_down):
    def _A_ref(x, k_cache, v_cache, wq, wo):
        B, Sq, D = x.shape
        H, Dh = 32, 192
        q = (lambda x, *d: x.transpose(*d))((x @ wq).reshape(B, Sq, H, Dh), 0, 2, 1, 3)
        scores = jnp.einsum("bhqd,bhkd->bhqk", q, k_cache) * (Dh ** -0.5)
        p = _softmax(scores, axis=-1)
        o = jnp.einsum("bhqk,bhkd->bhqd", p, v_cache)
        return (lambda x, *d: x.transpose(*d))(o, 0, 2, 1, 3).reshape(B, Sq, H * Dh) @ wo

    def _B_ref(x, w_r, w_gate, w_up, w_down):
        B, S, D = x.shape
        C = 1
        r = x @ w_r
        idx = jnp.argsort(-r, axis=-1)[:, :C]
        idx_e = jnp.repeat(idx.reshape(B, C, 1), D, axis=2)
        x_sel = jnp.take_along_axis(x, idx_e, axis=1)
        g = _silu(x_sel @ w_gate)
        u = x_sel @ w_up
        y = (g * u) @ w_down
        r_sel = _sigmoid(jnp.take_along_axis(r, idx, axis=1))
        y = y * r_sel.reshape(B, C, 1)
        b_off = (jnp.arange(B) * S).reshape(B, 1)
        flat_idx = (idx + b_off).reshape(B * C)
        zero = (x * 0.0).reshape(B * S, D)
        upd = _scatter_add(zero, flat_idx, y.reshape(B * C, D), axis=0)
        return x + upd.reshape(B, S, D)

    x = A_x
    h = x + _A_ref(_layernorm(x, axis=-1), A_k_cache, A_v_cache, A_wq, A_wo)
    h2 = h + _B_ref(_layernorm(h, axis=-1), B_w_r, B_w_gate, B_w_up, B_w_down)
    return h2
```

```python
import functools

import jax
import jax.numpy as jnp
import jax.experimental.pallas as pl
import jax.experimental.pallas.tpu as pltpu

_EPS = 1e-5
_TC = 1024
_TP = 256
_NH = 2


def _layernorm(x):
    m = jnp.mean(x, axis=-1, keepdims=True)
    d = x - m
    v = jnp.mean(d * d, axis=-1, keepdims=True)
    return d * jax.lax.rsqrt(v + _EPS)


def _bf16_round(x):
    return x.astype(jnp.bfloat16).astype(jnp.float32)


def _kernel(x_ref, wr_ref, kt_hbm, vt_hbm, wq_hbm, wo_hbm, wg_hbm, wu_hbm, wd_hbm,
            out_ref,
            buf, wq_v, wo_v, wg_v, wu_v, wd_v, q_s, s_s, o_s, sems, wsems,
            *, B, H, Dh, Sk, D):
    f32, bf16 = jnp.float32, jnp.bfloat16
    NC = Sk // _TC
    NP = _TC // _TP
    G = B * H

    def issue(src, g, j, slot):
        row = (g % B) * H + g // B
        for p in range(NP):
            col = pl.multiple_of(j * _TC + p * _TP, _TP)
            pltpu.make_async_copy(
                src.at[row, :, pl.ds(col, _TP)],
                buf.at[slot, :, pl.ds(p * _TP, _TP)],
                sems.at[slot],
            ).start(priority=p % 2)

    def wait(slot):
        pltpu.make_async_copy(buf.at[slot], buf.at[slot], sems.at[slot]).wait()

    wq_cp = pltpu.make_async_copy(wq_hbm, wq_v, wsems.at[0])
    wo_cp = pltpu.make_async_copy(wo_hbm, wo_v, wsems.at[1])
    wg_cp = pltpu.make_async_copy(wg_hbm, wg_v, wsems.at[2])
    wu_cp = pltpu.make_async_copy(wu_hbm, wu_v, wsems.at[3])
    wd_cp = pltpu.make_async_copy(wd_hbm, wd_v, wsems.at[4])

    wq_cp.start()

    def prologue(n, c):
        g = n // NC
        j = n % NC
        issue(kt_hbm, g, j, g * 2 * NC + j)
        issue(vt_hbm, g, j, g * 2 * NC + NC + j)
        return c
    jax.lax.fori_loop(0, NC, prologue, 0)
    wo_cp.start()
    if _NH > 1:
        jax.lax.fori_loop(NC, _NH * NC, prologue, 0)
    wg_cp.start()
    wu_cp.start()
    wd_cp.start()

    x = x_ref[...].astype(f32)
    xn = _layernorm(x).astype(bf16)
    wq_cp.wait()
    for hp in range(H // 2):
        q2 = jnp.dot(xn, wq_v[:, hp * 2 * Dh:(hp + 1) * 2 * Dh], preferred_element_type=f32)
        q2 = _bf16_round(q2)
        q_s[2 * hp] = q2[:, :Dh]
        q_s[2 * hp + 1] = q2[:, Dh:]

    scale = Dh ** -0.5

    def slab(g, acc):
        h = g // B
        b = g % B
        base = (g % _NH) * 2 * NC
        q = jnp.broadcast_to(q_s[h, pl.ds(b, 1), :], (8, Dh)).astype(bf16)

        def qk(j, m):
            slot = base + j
            wait(slot)
            s = jnp.dot(q, buf[slot], preferred_element_type=f32) * scale
            s_s[j] = s

            @pl.when(g + _NH < G)
            def _():
                issue(kt_hbm, g + _NH, j, slot)
            return jnp.maximum(m, s)
        m = jax.lax.fori_loop(0, NC, qk, jnp.full((8, _TC), -jnp.inf, f32))
        m = jnp.max(m, axis=-1, keepdims=True)

        def pv(j, c):
            l, o = c
            slot = base + NC + j
            p = jnp.exp(s_s[j] - m)
            wait(slot)
            o = o + jax.lax.dot_general(p.astype(bf16), buf[slot], (((1,), (1,)), ((), ())),
                                        preferred_element_type=f32)

            @pl.when(g + _NH < G)
            def _():
                issue(vt_hbm, g + _NH, j, slot)
            return l + p, o
        l, o = jax.lax.fori_loop(0, NC, pv, (jnp.zeros((8, _TC), f32), jnp.zeros((8, Dh), f32)))
        l = jnp.sum(l, axis=-1, keepdims=True)
        o = o / l
        rows = jax.lax.broadcasted_iota(jnp.int32, (8, Dh), 0)
        o = jnp.where(rows == b, o, 0.0).astype(bf16)

        @pl.when(g == 0)
        def _():
            wo_cp.wait()
        w = wo_v[pl.ds(pl.multiple_of(h * Dh, Dh), Dh), :]
        return acc + jnp.dot(o, w, preferred_element_type=f32)

    acc = jax.lax.fori_loop(0, G, slab, jnp.zeros((8, D), f32))
    hres = x + acc[:B]
    hn32 = _layernorm(hres)
    hn = hn32.astype(bf16)
    r = jnp.sum(hn.astype(f32) * wr_ref[...].astype(f32), axis=-1, keepdims=True)
    wg_cp.wait()
    gate = jnp.dot(hn, wg_v[...], preferred_element_type=f32)
    wu_cp.wait()
    up = jnp.dot(hn, wu_v[...], preferred_element_type=f32)
    act = (gate * jax.nn.sigmoid(gate) * up).astype(bf16)
    wd_cp.wait()
    y = jnp.dot(act, wd_v[...], preferred_element_type=f32) * jax.nn.sigmoid(r)
    upd = hn32 * 0.0 + y
    out_ref[...] = (hres + (hn32 + upd)).astype(out_ref.dtype)


@jax.jit
def pallas_sequential_preLN__mha_block_cached__moe_arch_mod__decode_kernel(
    A_x: jax.Array,
    A_k_cache: jax.Array,
    A_v_cache: jax.Array,
    A_wq: jax.Array,
    A_wo: jax.Array,
    B_x: jax.Array,
    B_w_r: jax.Array,
    B_w_gate: jax.Array,
    B_w_up: jax.Array,
    B_w_down: jax.Array,
):
    B, Sq, D = A_x.shape
    _, H, Sk, Dh = A_k_cache.shape
    F = B_w_gate.shape[1]
    kt = jnp.swapaxes(A_k_cache, 2, 3).reshape(B * H, Dh, Sk)
    vt = jnp.swapaxes(A_v_cache, 2, 3).reshape(B * H, Dh, Sk)
    nslots = _NH * 2 * (Sk // _TC)
    vmem = pl.BlockSpec(memory_space=pltpu.VMEM)
    hbm = pl.BlockSpec(memory_space=pl.ANY)
    out = pl.pallas_call(
        functools.partial(_kernel, B=B, H=H, Dh=Dh, Sk=Sk, D=D),
        in_specs=[vmem, vmem] + [hbm] * 7,
        out_specs=vmem,
        out_shape=jax.ShapeDtypeStruct((B, D), A_x.dtype),
        scratch_shapes=[
            pltpu.VMEM((nslots, Dh, _TC), jnp.bfloat16),
            pltpu.VMEM((D, H * Dh), jnp.bfloat16),
            pltpu.VMEM((H * Dh, D), jnp.bfloat16),
            pltpu.VMEM((D, F), jnp.bfloat16),
            pltpu.VMEM((D, F), jnp.bfloat16),
            pltpu.VMEM((F, D), jnp.bfloat16),
            pltpu.VMEM((H, B, Dh), jnp.float32),
            pltpu.VMEM((Sk // _TC, 8, _TC), jnp.float32),
            pltpu.VMEM((8, Dh), jnp.float32),
            pltpu.SemaphoreType.DMA((nslots,)),
            pltpu.SemaphoreType.DMA((5,)),
        ],
        compiler_params=pltpu.CompilerParams(vmem_limit_bytes=100 * 1024 * 1024),
    )(A_x.reshape(B, D), B_w_r.reshape(1, D), kt, vt, A_wq, A_wo, B_w_gate, B_w_up, B_w_down)
    return out.reshape(B, Sq, D)
```

```python
import functools

import jax
import jax.numpy as jnp
import jax.experimental.pallas as pl
import jax.experimental.pallas.tpu as pltpu

_EPS = 1e-5
_TC = 1024
_TP = 256
_NS = 16
_P0 = 0
_NAT = True
_DB = (0, 6, 10, 12)
_XP = (0, 1)
_WQ_ROWS = 8
_WO_ROWS = 64
_WG_ROWS = 32


def _layernorm(x):
    m = jnp.mean(x, axis=-1, keepdims=True)
    d = x - m
    v = jnp.mean(d * d, axis=-1, keepdims=True)
    return d * jax.lax.rsqrt(v + _EPS)


def _bf16_round(x):
    return x.astype(jnp.bfloat16).astype(jnp.float32)


def _kernel(x_hbm, wr_hbm, kt_hbm, vt_hbm, wq_hbm, wo_hbm, wg_hbm, wu_hbm, wd_hbm,
            out_ref,
            buf, x_v, wr_v, wq_v, wo_v, wg_v, wu_v, wd_v, q_s, s_s, sems, wsems, dsems,
            *, B, H, Dh, Sk, D, F):
    f32, bf16 = jnp.float32, jnp.bfloat16
    NC = Sk // _TC
    NP = _TC // _TP
    G = B * H
    ND = F // (2 * _WO_ROWS)

    def issue(src, g, j, slot):
        row = g if _NAT else (g % B) * H + g // B
        for p in range(NP):
            col = pl.multiple_of(j * _TC + p * _TP, _TP)
            pltpu.make_async_copy(
                src.at[row, :, pl.ds(col, _TP)],
                buf.at[slot, :, pl.ds(p * _TP, _TP)],
                sems.at[slot],
            ).start(priority=(p + _P0) % 2)

    def wait_all(ref, sem):
        pltpu.make_async_copy(ref, ref, sem).wait()

    def issue_pair(src, dst, rows, i, sem):
        for p in range(2):
            r = pl.multiple_of((2 * i + p) * rows, rows)
            pltpu.make_async_copy(src.at[pl.ds(r, rows), :], dst.at[pl.ds(r, rows), :],
                                  sem).start(priority=p)

    def issue_rows(src, dst, rows, sem):
        def body(i, c):
            issue_pair(src, dst, rows, i, sem)
            return c
        jax.lax.fori_loop(0, src.shape[0] // (2 * rows), body, 0)

    NG = D // (2 * _WG_ROWS)
    assert 2 * NG + ND == 2 * NC * (NP // 2)

    def issue_ffn(n):
        for k in range(NP // 2):
            i = n * (NP // 2) + k

            @pl.when(i < NG)
            def _():
                issue_pair(wg_hbm, wg_v, _WG_ROWS, i, wsems.at[4])

            @pl.when(jnp.logical_and(i >= NG, i < 2 * NG))
            def _():
                issue_pair(wu_hbm, wu_v, _WG_ROWS, i - NG, wsems.at[5])

            @pl.when(i >= 2 * NG)
            def _():
                issue_pair(wd_hbm, wd_v, _WO_ROWS, i - 2 * NG, dsems.at[i - 2 * NG])

    x_cp = pltpu.make_async_copy(x_hbm, x_v, wsems.at[0])
    wr_cp = pltpu.make_async_copy(wr_hbm, wr_v, wsems.at[1])
    x_cp.start(priority=_XP[0])
    wr_cp.start(priority=_XP[1])
    issue_rows(wq_hbm, wq_v, _WQ_ROWS, wsems.at[2])

    def issue_chunk(n):
        g = n // (2 * NC)
        jj = n % (2 * NC)
        slot = n % _NS

        @pl.when(jnp.logical_and(g < G, jj < NC))
        def _():
            issue(kt_hbm, g, jj, slot)

        @pl.when(jnp.logical_and(g < G, jj >= NC))
        def _():
            issue(vt_hbm, g, jj - NC, slot)

        @pl.when(g == G)
        def _():
            issue_ffn(jj)

    def prologue(n, c):
        issue_chunk(n)
        return c
    jax.lax.fori_loop(0, min(_NS, 2 * NC), prologue, 0)

    x_cp.wait()
    x = x_v[...].astype(f32)
    xn = _layernorm(x).astype(bf16)
    wait_all(wq_v, wsems.at[2])
    for hp in range(H // 2):
        q2 = jnp.dot(xn, wq_v[:, hp * 2 * Dh:(hp + 1) * 2 * Dh], preferred_element_type=f32)
        q2 = _bf16_round(q2)
        q_s[2 * hp] = q2[:, :Dh]
        q_s[2 * hp + 1] = q2[:, Dh:]

    issue_rows(wo_hbm, wo_v, _WO_ROWS, wsems.at[3])
    if _NS > 2 * NC:
        jax.lax.fori_loop(2 * NC, _NS, prologue, 0)

    scale = Dh ** -0.5

    def slab(g, acc):
        h = g % H if _NAT else g // B
        b = g // H if _NAT else g % B
        base = g * 2 * NC
        q = jnp.broadcast_to(q_s[h, pl.ds(b, 1), :], (8, Dh)).astype(bf16)

        def qk(j, m):
            n = base + j
            slot = n % _NS
            wait_all(buf.at[slot], sems.at[slot])
            s = jnp.dot(q, buf[slot], preferred_element_type=f32) * scale
            s_s[j] = s
            issue_chunk(n + _NS)
            return jnp.maximum(m, s)
        m = jax.lax.fori_loop(0, NC, qk, jnp.full((8, _TC), -jnp.inf, f32))
        m = jnp.max(m, axis=-1, keepdims=True)

        def pv(j, c):
            l, o = c
            n = base + NC + j
            slot = n % _NS
            p = jnp.exp(s_s[j] - m)
            wait_all(buf.at[slot], sems.at[slot])
            o = o + jax.lax.dot_general(p.astype(bf16), buf[slot], (((1,), (1,)), ((), ())),
                                        preferred_element_type=f32)
            issue_chunk(n + _NS)
            return l + p, o
        l, o = jax.lax.fori_loop(0, NC, pv, (jnp.zeros((8, _TC), f32), jnp.zeros((8, Dh), f32)))
        l = jnp.sum(l, axis=-1, keepdims=True)
        o = o / l
        rows = jax.lax.broadcasted_iota(jnp.int32, (8, Dh), 0)
        o = jnp.where(rows == b, o, 0.0).astype(bf16)

        @pl.when(g == 0)
        def _():
            wait_all(wo_v, wsems.at[3])
        w = wo_v[pl.ds(pl.multiple_of(h * Dh, Dh), Dh), :]
        return acc + jnp.dot(o, w, preferred_element_type=f32)

    acc = jax.lax.fori_loop(0, G, slab, jnp.zeros((8, D), f32))
    if _NS < 2 * NC:
        jax.lax.fori_loop(2 * NC * G + _NS, 2 * NC * (G + 1), prologue, 0)
    hres = x + acc[:B]
    hn32 = _layernorm(hres)
    hn = hn32.astype(bf16)
    wr_cp.wait()
    r = jnp.sum(hn.astype(f32) * wr_v[...].astype(f32).reshape(1, D), axis=-1, keepdims=True)
    rgate = jax.nn.sigmoid(r)
    wait_all(wg_v, wsems.at[4])
    gate = jnp.dot(hn, wg_v[...], preferred_element_type=f32)
    wait_all(wu_v, wsems.at[5])
    up = jnp.dot(hn, wu_v[...], preferred_element_type=f32)
    act = (gate * jax.nn.sigmoid(gate) * up).astype(bf16)
    y = jnp.zeros((B, D), f32)
    R = 2 * _WO_ROWS
    for lo, hi in zip(_DB[:-1], _DB[1:]):
        for i in range(lo, hi):
            wait_all(wd_v.at[pl.ds(i * R, R), :], dsems.at[i])
        y = y + jnp.dot(act[:, lo * R:hi * R], wd_v[lo * R:hi * R, :], preferred_element_type=f32)
    upd = hn32 * 0.0 + y * rgate
    out_ref[...] = (hres + (hn32 + upd)).astype(out_ref.dtype)


@jax.jit
def pallas_sequential_preLN__mha_block_cached__moe_arch_mod__decode_kernel(
    A_x: jax.Array,
    A_k_cache: jax.Array,
    A_v_cache: jax.Array,
    A_wq: jax.Array,
    A_wo: jax.Array,
    B_x: jax.Array,
    B_w_r: jax.Array,
    B_w_gate: jax.Array,
    B_w_up: jax.Array,
    B_w_down: jax.Array,
):
    B, Sq, D = A_x.shape
    _, H, Sk, Dh = A_k_cache.shape
    F = B_w_gate.shape[1]
    kt = jnp.swapaxes(A_k_cache, 2, 3).reshape(B * H, Dh, Sk)
    vt = jnp.swapaxes(A_v_cache, 2, 3).reshape(B * H, Dh, Sk)
    nslots = _NS
    out = pl.pallas_call(
        functools.partial(_kernel, B=B, H=H, Dh=Dh, Sk=Sk, D=D, F=F),
        in_specs=[pl.BlockSpec(memory_space=pl.ANY)] * 9,
        out_specs=pl.BlockSpec(memory_space=pltpu.VMEM),
        out_shape=jax.ShapeDtypeStruct((B, D), A_x.dtype),
        scratch_shapes=[
            pltpu.VMEM((nslots, Dh, _TC), jnp.bfloat16),
            pltpu.VMEM((B, D), jnp.bfloat16),
            pltpu.VMEM((D,), jnp.bfloat16),
            pltpu.VMEM((D, H * Dh), jnp.bfloat16),
            pltpu.VMEM((H * Dh, D), jnp.bfloat16),
            pltpu.VMEM((D, F), jnp.bfloat16),
            pltpu.VMEM((D, F), jnp.bfloat16),
            pltpu.VMEM((F, D), jnp.bfloat16),
            pltpu.VMEM((H, B, Dh), jnp.float32),
            pltpu.VMEM((Sk // _TC, 8, _TC), jnp.float32),
            pltpu.SemaphoreType.DMA((nslots,)),
            pltpu.SemaphoreType.DMA((6,)),
            pltpu.SemaphoreType.DMA((F // (2 * _WO_ROWS),)),
        ],
        compiler_params=pltpu.CompilerParams(vmem_limit_bytes=100 * 1024 * 1024),
    )(A_x.reshape(B, D), B_w_r, kt, vt, A_wq, A_wo, B_w_gate, B_w_up, B_w_down)
    return out.reshape(B, Sq, D)
```

```python
import functools

import jax
import jax.numpy as jnp
import jax.experimental.pallas as pl
import jax.experimental.pallas.tpu as pltpu

_EPS = 1e-5
_TC = 2048
_TP = 256
_NS = 16
_WR = 160
_TR = 64
_DB = (0, 6, 10, 12)


def _layernorm(x):
    m = jnp.mean(x, axis=-1, keepdims=True)
    d = x - m
    v = jnp.mean(d * d, axis=-1, keepdims=True)
    return d * jax.lax.rsqrt(v + _EPS)


def _wait_all(ref, sem):
    pltpu.make_async_copy(ref, ref, sem).wait()


def _issue_strip(src, dst, i, sem):
    cols = pl.ds(pl.multiple_of(i * _TP, _TP), _TP)
    for p in range(src.shape[0] // _WR):
        rows = pl.ds(p * _WR, _WR)
        pltpu.make_async_copy(src.at[rows, cols], dst.at[rows, cols], sem).start(priority=p % 2)


def _issue_band(src, dst, i, sem):
    for p in range(2):
        rows = pl.ds(pl.multiple_of((2 * i + p) * _TR, _TR), _TR)
        pltpu.make_async_copy(src.at[rows, :], dst.at[rows, :], sem).start(priority=p)


def _loop(lo, hi, fn):
    def body(i, c):
        fn(i)
        return c
    jax.lax.fori_loop(lo, hi, body, 0)


def _kernel(x_hbm, wr_hbm, kt_hbm, vt_hbm, wq_hbm, wo_hbm, wg_hbm, wu_hbm, wd_hbm,
            out_ref,
            buf, x_v, wr_v, wq_v, wo_v, wg_v, wu_v, wd_v, q_s, s_s, sems, wsems, dsems,
            *, B, H, Dh, Sk, D, F):
    f32, bf16 = jnp.float32, jnp.bfloat16
    NC = Sk // _TC
    G = B * H
    NKV = 2 * NC * G
    NG = F // _TP
    ND = F // (2 * _TR)
    NF = 2 * NG + ND // 2

    def issue_kv(src, g, j, slot):
        for p in range(_TC // _TP):
            col = pl.multiple_of(j * _TC + p * _TP, _TP)
            pltpu.make_async_copy(
                src.at[g, :, pl.ds(col, _TP)],
                buf.at[slot, :, pl.ds(p * _TP, _TP)],
                sems.at[slot],
            ).start(priority=p % 2)

    def issue_ffn(i):
        @pl.when(i < NG)
        def _():
            _issue_strip(wg_hbm, wg_v, i, wsems.at[4])

        @pl.when(jnp.logical_and(i >= NG, i < 2 * NG))
        def _():
            _issue_strip(wu_hbm, wu_v, i - NG, wsems.at[5])

        @pl.when(i >= 2 * NG)
        def _():
            for k in range(2):
                band = 2 * (i - 2 * NG) + k
                _issue_band(wd_hbm, wd_v, band, dsems.at[band])

    def issue(n):
        g = n // (2 * NC)
        jj = n % (2 * NC)
        slot = n % _NS

        @pl.when(jnp.logical_and(n < NKV, jj < NC))
        def _():
            issue_kv(kt_hbm, g, jj, slot)

        @pl.when(jnp.logical_and(n < NKV, jj >= NC))
        def _():
            issue_kv(vt_hbm, g, jj - NC, slot)

        @pl.when(jnp.logical_and(n >= NKV, n < NKV + NF))
        def _():
            issue_ffn(n - NKV)

    x_cp = pltpu.make_async_copy(x_hbm, x_v, wsems.at[0])
    wr_cp = pltpu.make_async_copy(wr_hbm, wr_v, wsems.at[1])
    x_cp.start()
    wr_cp.start(priority=1)
    _loop(0, H * Dh // _TP, lambda i: _issue_strip(wq_hbm, wq_v, i, wsems.at[2]))
    first = min(_NS, 2 * NC)
    _loop(0, first, issue)

    x_cp.wait()
    x = x_v[...].astype(f32)
    xn = _layernorm(x).astype(bf16)
    _wait_all(wq_v, wsems.at[2])
    for hp in range(H // 2):
        q2 = jnp.dot(xn, wq_v[:, hp * 2 * Dh:(hp + 1) * 2 * Dh], preferred_element_type=f32)
        q_s[2 * hp] = q2[:, :Dh]
        q_s[2 * hp + 1] = q2[:, Dh:]

    _loop(0, H * Dh // (2 * _TR), lambda i: _issue_band(wo_hbm, wo_v, i, wsems.at[3]))
    if _NS > first:
        _loop(first, _NS, issue)

    scale = Dh ** -0.5

    def slab(tail, g, acc):
        b = g // H
        h = g % H
        base = g * 2 * NC
        q = jnp.broadcast_to(q_s[h, pl.ds(b, 1), :], (8, Dh)).astype(bf16)

        def refill(phase, j, slot):
            if tail:
                issue(base + phase * NC + j + _NS)
            else:
                ahead = phase + _NS // NC
                issue_kv((kt_hbm, vt_hbm)[ahead % 2], g + ahead // 2, j, slot)

        def qk(j, m):
            slot = base % _NS + j
            _wait_all(buf.at[slot], sems.at[slot])
            s = jnp.dot(q, buf[slot], preferred_element_type=f32) * scale
            s_s[j] = s
            refill(0, j, slot)
            return jnp.maximum(m, s)
        m = jax.lax.fori_loop(0, NC, qk, jnp.full((8, _TC), -jnp.inf, f32))
        m = jnp.max(m, axis=-1, keepdims=True)

        def pv(j, c):
            l, o = c
            slot = (base + NC) % _NS + j
            p = jnp.exp(s_s[j] - m)
            _wait_all(buf.at[slot], sems.at[slot])
            o = o + jax.lax.dot_general(p.astype(bf16), buf[slot], (((1,), (1,)), ((), ())),
                                        preferred_element_type=f32)
            refill(1, j, slot)
            return l + p, o
        l, o = jax.lax.fori_loop(0, NC, pv, (jnp.zeros((8, _TC), f32), jnp.zeros((8, Dh), f32)))
        o = o / jnp.sum(l, axis=-1, keepdims=True)
        rows = jax.lax.broadcasted_iota(jnp.int32, (8, Dh), 0)
        o = jnp.where(rows == b, o, 0.0).astype(bf16)

        @pl.when(g == 0)
        def _():
            _wait_all(wo_v, wsems.at[3])
        w = wo_v[pl.ds(pl.multiple_of(h * Dh, Dh), Dh), :]
        return acc + jnp.dot(o, w, preferred_element_type=f32)

    assert _NS % NC == 0
    steady = G - (_NS // NC + 1) // 2
    acc = jax.lax.fori_loop(0, steady, functools.partial(slab, False), jnp.zeros((8, D), f32))
    acc = jax.lax.fori_loop(steady, G, functools.partial(slab, True), acc)
    if _NS < NF:
        _loop(NKV + _NS, NKV + NF, issue)

    hres = x + acc[:B]
    hn32 = _layernorm(hres)
    hn = hn32.astype(bf16)
    wr_cp.wait()
    r = jnp.sum(hn.astype(f32) * wr_v[...].astype(f32).reshape(1, D), axis=-1, keepdims=True)
    rgate = jax.nn.sigmoid(r)
    _wait_all(wg_v, wsems.at[4])
    gate = jnp.dot(hn, wg_v[...], preferred_element_type=f32)
    gate = gate * jax.nn.sigmoid(gate)
    _wait_all(wu_v, wsems.at[5])
    act = (gate * jnp.dot(hn, wu_v[...], preferred_element_type=f32)).astype(bf16)
    y = jnp.zeros((B, D), f32)
    R = 2 * _TR
    assert _DB[0] == 0 and _DB[-1] == ND
    for lo, hi in zip(_DB[:-1], _DB[1:]):
        for i in range(lo, hi):
            _wait_all(wd_v.at[pl.ds(i * R, R), :], dsems.at[i])
        y = y + jnp.dot(act[:, lo * R:hi * R], wd_v[lo * R:hi * R, :], preferred_element_type=f32)
    upd = hn32 * 0.0 + y * rgate
    out_ref[...] = (hres + (hn32 + upd)).astype(out_ref.dtype)


@jax.jit
def pallas_sequential_preLN__mha_block_cached__moe_arch_mod__decode_kernel(
    A_x: jax.Array,
    A_k_cache: jax.Array,
    A_v_cache: jax.Array,
    A_wq: jax.Array,
    A_wo: jax.Array,
    B_x: jax.Array,
    B_w_r: jax.Array,
    B_w_gate: jax.Array,
    B_w_up: jax.Array,
    B_w_down: jax.Array,
):
    B, Sq, D = A_x.shape
    _, H, Sk, Dh = A_k_cache.shape
    F = B_w_gate.shape[1]
    kt = jnp.swapaxes(A_k_cache, 2, 3).reshape(B * H, Dh, Sk)
    vt = jnp.swapaxes(A_v_cache, 2, 3).reshape(B * H, Dh, Sk)
    out = pl.pallas_call(
        functools.partial(_kernel, B=B, H=H, Dh=Dh, Sk=Sk, D=D, F=F),
        in_specs=[pl.BlockSpec(memory_space=pl.ANY)] * 9,
        out_specs=pl.BlockSpec(memory_space=pltpu.VMEM),
        out_shape=jax.ShapeDtypeStruct((B, D), A_x.dtype),
        scratch_shapes=[
            pltpu.VMEM((_NS, Dh, _TC), jnp.bfloat16),
            pltpu.VMEM((B, D), jnp.bfloat16),
            pltpu.VMEM((D,), jnp.bfloat16),
            pltpu.VMEM((D, H * Dh), jnp.bfloat16),
            pltpu.VMEM((H * Dh, D), jnp.bfloat16),
            pltpu.VMEM((D, F), jnp.bfloat16),
            pltpu.VMEM((D, F), jnp.bfloat16),
            pltpu.VMEM((F, D), jnp.bfloat16),
            pltpu.VMEM((H, B, Dh), jnp.float32),
            pltpu.VMEM((Sk // _TC, 8, _TC), jnp.float32),
            pltpu.SemaphoreType.DMA((_NS,)),
            pltpu.SemaphoreType.DMA((6,)),
            pltpu.SemaphoreType.DMA((F // (2 * _TR),)),
        ],
        compiler_params=pltpu.CompilerParams(vmem_limit_bytes=100 * 1024 * 1024),
    )(A_x.reshape(B, D), B_w_r, kt, vt, A_wq, A_wo, B_w_gate, B_w_up, B_w_down)
    return out.reshape(B, Sq, D)
```
